```python
import os as _os
_os.environ.setdefault("JAX_PLATFORMS", "cpu")
import jax
import jax.numpy as jnp

def _softmax(x, axis=-1):
    return jax.nn.softmax(x, axis=axis)
def _gelu(x):
    return jax.nn.gelu(x, approximate=True)
def _silu(x):
    return jax.nn.silu(x)
def _sigmoid(x):
    return jax.nn.sigmoid(x)
def _layernorm(x, axis=-1, eps=1e-5):
    m = jnp.mean(x, axis=axis, keepdims=True)
    v = jnp.var(x, axis=axis, keepdims=True)
    return (x - m) / jnp.sqrt(v + eps)
def _scatter_add(tgt, idx, src, axis=0):
    return tgt.at[idx].add(src)
def _segment_sum(src, seg, n):
    return jax.ops.segment_sum(src, seg, n)
class _Rng:
    def __init__(self, key):
        self._k = key
    def _next(self):
        self._k, sub = jax.random.split(self._k)
        return sub
    def normal(self, shape):
        return jax.random.normal(self._next(), shape, dtype=jnp.bfloat16)
    def randint(self, lo, hi, shape):
        return jax.random.randint(self._next(), shape, lo, hi, dtype=jnp.int32)
    def uniform(self, shape, lo=0.0, hi=1.0):
        return jax.random.uniform(self._next(), shape, jnp.bfloat16, lo, hi)
    def permutation(self, n):
        return jax.random.permutation(self._next(), n)


kernel_name = 'concat_heads__gqa_block_cached__mha_block_cached__near_ridge'

def setup_inputs():
    _rng = _Rng(jax.random.key(int.from_bytes(__import__("os").urandom(4), "little")))
    _w = (lambda a: (lambda t: t.astype(jnp.bfloat16) if jnp.issubdtype(t.dtype, jnp.floating) else t)(jnp.asarray(a)))
    def _A_setup():
        B, Sq, D = 8, 48, 512
        Hq, Hkv, Sk, Dh = 32, 8, 1024, 128
        assert Hq % Hkv == 0, (Hq, Hkv)
        return {
            "x": _w((lambda *s: _rng.normal(s) * 0.8)(B, Sq, D)),
            "k_cache": _w((lambda *s: _rng.normal(s) * 0.8)(B, Hkv, Sk, Dh)),
            "v_cache": _w((lambda *s: _rng.normal(s) * 0.05)(B, Hkv, Sk, Dh)),
            "wq": _w((lambda *s: _rng.normal(s) * 0.8)(D, Hq * Dh) * (D ** -0.5)),
            "wo": _w((lambda *s: _rng.normal(s) * 0.05)(Hq * Dh, D) * ((Hq * Dh) ** -0.5)),
        }
    _A_in = _A_setup()

    def _B_setup():
        B, Sq, D = 8, 48, 512
        H, Sk, Dh = 32, 1024, 128
        return {
            "x": _w((lambda *s: _rng.normal(s) * 0.8)(B, Sq, D)),
            "k_cache": _w((lambda *s: _rng.normal(s) * 0.8)(B, H, Sk, Dh)),
            "v_cache": _w((lambda *s: _rng.normal(s) * 0.05)(B, H, Sk, Dh)),
            "wq": _w((lambda *s: _rng.normal(s) * 0.8)(D, H * Dh) * (D ** -0.5)),
            "wo": _w((lambda *s: _rng.normal(s) * 0.05)(H * Dh, D) * ((H * Dh) ** -0.5)),
        }
    _B_in = _B_setup()

    return {
        "A_x": _A_in["x"],
        "A_k_cache": _A_in["k_cache"],
        "A_v_cache": _A_in["v_cache"],
        "A_wq": _A_in["wq"],
        "A_wo": _A_in["wo"],
        "B_x": _B_in["x"],
        "B_k_cache": _B_in["k_cache"],
        "B_v_cache": _B_in["v_cache"],
        "B_wq": _B_in["wq"],
        "B_wo": _B_in["wo"],
    }

def reference(A_x, A_k_cache, A_v_cache, A_wq, A_wo, B_x, B_k_cache, B_v_cache, B_wq, B_wo):
    def _A_ref(x, k_cache, v_cache, wq, wo):
        B, Sq, D = x.shape
        Hq, Dh = 32, 128
        Hkv = k_cache.shape[1]
        rep = Hq // Hkv
        q = (lambda x, *d: x.transpose(*d))((x @ wq).reshape(B, Sq, Hq, Dh), 0, 2, 1, 3)
        k = jnp.repeat(k_cache, rep, axis=1)
        v = jnp.repeat(v_cache, rep, axis=1)
        scores = jnp.einsum("bhqd,bhkd->bhqk", q, k) * (Dh ** -0.5)
        p = _softmax(scores, axis=-1)
        o = jnp.einsum("bhqk,bhkd->bhqd", p, v)
        return (lambda x, *d: x.transpose(*d))(o, 0, 2, 1, 3).reshape(B, Sq, Hq * Dh) @ wo

    def _B_ref(x, k_cache, v_cache, wq, wo):
        B, Sq, D = x.shape
        H, Dh = 32, 128
        q = (lambda x, *d: x.transpose(*d))((x @ wq).reshape(B, Sq, H, Dh), 0, 2, 1, 3)
        scores = jnp.einsum("bhqd,bhkd->bhqk", q, k_cache) * (Dh ** -0.5)
        p = _softmax(scores, axis=-1)
        o = jnp.einsum("bhqk,bhkd->bhqd", p, v_cache)
        return (lambda x, *d: x.transpose(*d))(o, 0, 2, 1, 3).reshape(B, Sq, H * Dh) @ wo

    a = _A_ref(A_x, A_k_cache, A_v_cache, A_wq, A_wo)
    b = _B_ref(B_x, B_k_cache, B_v_cache, B_wq, B_wo)
    return jnp.concatenate([a, b], axis=-1)
```

```python
import functools
import math

import jax
import jax.numpy as jnp
from jax import lax
import jax.experimental.pallas as pl
import jax.experimental.pallas.tpu as pltpu

MiB = 1 << 20
NB, SQ, D, DH, SK = 8, 48, 512, 128, 1024
G, REP = 8, 4
M = NB * SQ
QSCALE = DH ** -0.5 * math.log2(math.e)

NT = (((1,), (1,)), ((), ()))


def _attend(q, k, v):
    s = lax.dot_general(q, k, NT, preferred_element_type=jnp.float32)
    m = jnp.max(s, axis=-1, keepdims=True)
    p = jnp.exp2(s - m)
    l = jnp.sum(p, axis=-1, keepdims=True)
    o = jnp.dot(p.astype(jnp.bfloat16), v, preferred_element_type=jnp.float32)
    return (o * (1.0 / l)).astype(jnp.bfloat16)


def make(nslots=3, look=2, rows=128, stagger=2, compute=True, dma=True):
    assert look < nslots or (look == nslots)
    nj = SK // rows

    def kernel(xa_h, ka_h, va_h, wqa_h, woa_h, xb_h, kb_h, vb_h, wqb_h, wob_h, out_h,
               x_v, wq_v, wo_v, ka_v, va_v, kb_v, vb_v, q_v, o_v, acc_v, out_v,
               sem_w, sem_kv, sem_out):
        def start_kv(s, slot):
            g = s // NB
            b = s % NB
            for j in range(nj):
                for h in range(REP):
                    for w in range(2):
                        jj = (j + stagger * (2 * h + w)) % nj
                        src, dst = ((kb_h, kb_v), (vb_h, vb_v))[w]
                        pltpu.make_async_copy(
                            src.at[b, g * REP + h, pl.ds(jj * rows, rows)],
                            dst.at[slot, h, pl.ds(jj * rows, rows)],
                            sem_kv.at[slot * 4 + 2 + w]).start(priority=w)
                for w in range(2):
                    src, dst = ((ka_h, ka_v), (va_h, va_v))[w]
                    pltpu.make_async_copy(
                        src.at[b, g, pl.ds(j * rows, rows)],
                        dst.at[slot, pl.ds(j * rows, rows)],
                        sem_kv.at[slot * 4 + w]).start(priority=w)

        def wait_all(ref, sem):
            pltpu.make_async_copy(ref, ref, sem).wait()

        for i, src in enumerate((xa_h, xb_h)):
            pltpu.make_async_copy(src, x_v.at[i], sem_w.at[0]).start(priority=i)

        @pl.loop(0, D // 16)
        def _(r):
            r0 = pl.multiple_of(r * 16, 16)
            for c in range(4):
                for i, src in enumerate((wqa_h, wqb_h)):
                    pltpu.make_async_copy(
                        src.at[pl.ds(r0, 16), pl.ds(c * 1024, 1024)],
                        wq_v.at[i, pl.ds(r0, 16), pl.ds(c * 1024, 1024)],
                        sem_w.at[1]).start(priority=i)

        if dma:
            for s in range(look):
                start_kv(s, s % nslots)

        @pl.loop(0, G * REP * DH // 32)
        def _(r):
            r0 = pl.multiple_of(r * 32, 32)
            for i, src in enumerate((woa_h, wob_h)):
                pltpu.make_async_copy(
                    src.at[pl.ds(r0, 32)], wo_v.at[i, pl.ds(r0, 32)],
                    sem_w.at[2]).start(priority=i)

        def q_piece(g, t):
            i = t // REP
            j = t % REP
            col = pl.multiple_of((g * REP + j) * DH, DH)
            q = jnp.dot(x_v[i], wq_v[i, :, pl.ds(col, DH)], preferred_element_type=jnp.float32)
            q_v[g % 2, t] = (q * QSCALE).astype(jnp.bfloat16)

        def o_piece(g, t, first):
            i = t // REP
            n = t % REP
            lhs = jnp.concatenate([o_v[g % 2, i * REP + j] for j in range(REP)], axis=1)
            row = pl.multiple_of(g * REP * DH, REP * DH)
            col = pl.multiple_of(n * DH, DH)
            y = jnp.dot(lhs, wo_v[i, pl.ds(row, REP * DH), pl.ds(col, DH)],
                        preferred_element_type=jnp.float32)
            if first:
                acc_v[t] = y
            else:
                acc_v[t] += y

        wait_all(x_v, sem_w.at[0])
        wait_all(wq_v, sem_w.at[1])
        if compute:
            @pl.loop(0, NB)
            def _(t):
                q_piece(0, t)
        acc_v[...] = jnp.zeros_like(acc_v)
        wait_all(wo_v, sem_w.at[2])

        def step(s, do_q, do_o, do_start):
            g = s // NB
            b = s % NB
            slot = s % nslots
            if dma:
                wait_all(ka_v.at[slot], sem_kv.at[slot * 4 + 0])
                wait_all(va_v.at[slot], sem_kv.at[slot * 4 + 1])
                wait_all(kb_v.at[slot], sem_kv.at[slot * 4 + 2])
                wait_all(vb_v.at[slot], sem_kv.at[slot * 4 + 3])
                if do_start:
                    start_kv(s + look, (s + look) % nslots)
            if not compute:
                return
            r0 = pl.multiple_of(b * SQ, SQ)
            par = g % 2
            qa = jnp.concatenate([q_v[par, j, pl.ds(r0, SQ), :] for j in range(REP)], axis=0)
            oa = _attend(qa, ka_v[slot], va_v[slot])
            for j in range(REP):
                o_v[par, j, pl.ds(r0, SQ), :] = oa[j * SQ:(j + 1) * SQ]
            for j in range(REP):
                ob = _attend(q_v[par, REP + j, pl.ds(r0, SQ), :], kb_v[slot, j], vb_v[slot, j])
                o_v[par, REP + j, pl.ds(r0, SQ), :] = ob
            if do_q:
                q_piece(g + 1, b)
            if do_o:
                o_piece(g - 1, b, False)

        n = G * NB

        @pl.loop(0, NB)
        def _(s):
            step(s, True, False, True)

        @pl.loop(NB, n - NB)
        def _(s):
            step(s, True, True, True)

        @pl.loop(n - NB, n - look)
        def _(s):
            step(s, False, True, True)

        @pl.loop(n - look, n)
        def _(s):
            step(s, False, True, False)

        if compute:
            @pl.loop(0, NB)
            def _(t):
                o_piece(G - 1, t, False)
        for t in range(NB):
            out_v[:, t * DH:(t + 1) * DH] = acc_v[t].astype(jnp.bfloat16)
        cp = pltpu.make_async_copy(out_v, out_h, sem_out)
        cp.start()
        cp.wait()

    def fn(A_x, A_k, A_v, A_wq, A_wo, B_x, B_k, B_v, B_wq, B_wo):
        bf = jnp.bfloat16
        out = pl.pallas_call(
            kernel,
            in_specs=[pl.BlockSpec(memory_space=pl.ANY)] * 10,
            out_specs=pl.BlockSpec(memory_space=pl.ANY),
            out_shape=jax.ShapeDtypeStruct((M, 2 * D), bf),
            scratch_shapes=[
                pltpu.VMEM((2, M, D), bf),
                pltpu.VMEM((2, D, G * REP * DH), bf),
                pltpu.VMEM((2, G * REP * DH, D), bf),
                pltpu.VMEM((nslots, SK, DH), bf),
                pltpu.VMEM((nslots, SK, DH), bf),
                pltpu.VMEM((nslots, REP, SK, DH), bf),
                pltpu.VMEM((nslots, REP, SK, DH), bf),
                pltpu.VMEM((2, 2 * REP, M, DH), bf),
                pltpu.VMEM((2, 2 * REP, M, DH), bf),
                pltpu.VMEM((2 * REP, M, DH), jnp.float32),
                pltpu.VMEM((M, 2 * D), bf),
                pltpu.SemaphoreType.DMA((3,)),
                pltpu.SemaphoreType.DMA((nslots * 4,)),
                pltpu.SemaphoreType.DMA(()),
            ],
            compiler_params=pltpu.CompilerParams(vmem_limit_bytes=100 * MiB),
        )(A_x.reshape(M, D), A_k, A_v, A_wq, A_wo, B_x.reshape(M, D), B_k, B_v, B_wq, B_wo)
        return out.reshape(NB, SQ, 2 * D)
    return fn


_kernel_fn = make()


@jax.jit
def pallas_concat_heads__gqa_block_cached__mha_block_cached__near_ridge_kernel(
    A_x, A_k_cache, A_v_cache, A_wq, A_wo, B_x, B_k_cache, B_v_cache, B_wq, B_wo
):
    return _kernel_fn(A_x, A_k_cache, A_v_cache, A_wq, A_wo, B_x, B_k_cache, B_v_cache, B_wq, B_wo)
```

```python
import contextlib
import functools
import math

import numpy as np
import jax
import jax.numpy as jnp
from jax import lax
import jax.experimental.pallas as pl
import jax.experimental.pallas.tpu as pltpu

MiB = 1 << 20
NB, SQ, D, DH, SK = 8, 48, 512, 128, 1024
G, REP = 8, 4
GW = REP * DH
HW = G * GW
QSCALE = DH ** -0.5 * math.log2(math.e)
NT = (((1,), (1,)), ((), ()))
bf16, f32, u32 = jnp.bfloat16, jnp.float32, jnp.uint32
CH = 128
NCH = SK // CH

ORDER_AB = "Qb Qa K0 K1 S0 Ka S1 V0 K2 V1 Sa K3 S2 Va S3 V2 V3 Oa Ob"
ORDER_A = "Qa Ka Sa Va Oa"
ORDER_B = "Qb K0 K1 K2 K3 S0 S1 S2 S3 V0 V1 V2 V3 Ob"


def default_pattern(stagger=2):
    q = ([], [])
    for j in range(NCH):
        for h in range(REP):
            for w in range(2):
                q[w].append((2 + w, h, (j + stagger * (2 * h + w)) % NCH))
        for w in range(2):
            q[w].append((w, 0, j))
    return q


def last_pattern(stagger=2):
    ks = [(2, h, (j + stagger * 2 * h) % NCH) for j in range(NCH) for h in range(REP)]
    vs = [(3, h, j) for h in range(REP) for j in range(NCH)]
    return ks, vs


def make(ahead=2, x0=15, x1=40, pattern=None, lastpat=None, compute=True, prof=False,
         flags=None, vgroups=((0, 1), (2,), (3,)), out_mode="each", order=ORDER_AB, nslots=3,
         out_prio=1, wstreams=1, wstag=0, early_q=True, xl=None, table=False, out_rows=0, fin_prio=0, hmap='c', mids=()):
    pattern = pattern or default_pattern()
    lastpat = lastpat or last_pattern()
    n = NB * G
    scope = (lambda nm: jax.named_scope(nm)) if prof else (lambda nm: contextlib.nullcontext())
    vgroup_of = {h: i for i, hs in enumerate(vgroups) for h in hs}
    cut = (x0, x1)
    bonly = tuple([e for e in q if e[0] >= 2] for q in pattern)
    cut_b = xl or tuple(max(0, x - 8) for x in cut)

    def kernel(*refs):
        if table:
            tab, refs = refs[0], refs[1:]
        (xa_h, ka_h, va_h, wqa_h, woa_h, xb_h, kb_h, vb_h, wqb_h, wob_h, out_h,
         x_v, wq_v, wo_v, kva_v, kvb_v, acc_v, out_v, sems) = refs

        class Sub:
            def __init__(self, base):
                self.base = base
                self.at = self

            def __getitem__(self, i):
                return sems.at[self.base + i]
        sem_w, sem_a, sem_b, sem_l = Sub(1), Sub(4), Sub(4 + nslots), Sub(4 + 2 * nslots)
        sem_out = sems.at[0]
        x_h, wq_h, wo_h = (xa_h, xb_h), (wqa_h, wqb_h), (woa_h, wob_h)

        def load(ref):
            return pltpu.bitcast(ref.bitcast(u32)[...], bf16)

        def wait_all(ref, sem):
            pltpu.make_async_copy(ref, ref, sem).wait()

        def kv_copies(t, items, last=False, tab_at=None):
            ua = t + ahead
            res = []
            for k, (a, h, j) in enumerate(items):
                if tab_at is not None:
                    code = tab[tab_at + k]
                    h = code >> 3
                    rows = pl.ds(pl.multiple_of((code & 7) * CH, CH), CH)
                else:
                    rows = pl.ds(j * CH, CH)
                if a < 2:
                    cp = pltpu.make_async_copy((ka_h, va_h)[a].at[ua // G, ua % G, rows],
                                               kva_v.at[ua % nslots, a, rows], sem_a.at[ua % nslots])
                else:
                    sem = sem_l.at[vgroup_of[h]] if last and a == 3 else sem_b.at[t % nslots]
                    bb, hh = {'c': (t // G, (t % G) * REP + h), 's': (t // G, (t % G) + G * h),
                              'x4': ((t // 32) * 4 + h, t % 32),
                              'x2': ((t // 16) * 2 + h // 2, (t % 16) + 16 * (h % 2))}[hmap]
                    cp = pltpu.make_async_copy((kb_h, vb_h)[a - 2].at[bb, hh, rows],
                                               kvb_v.at[t % nslots, a - 2, h, rows], sem)
                res.append(cp)
            return res

        def start(q0, q1):
            for k in range(max(len(q0), len(q1))):
                for p, q in enumerate((q0, q1)):
                    if k < len(q):
                        q[k].start(priority=p)

        def part(t, kind, first):
            if kind is None:
                return [], []
            pat = {"ab": pattern, "b": bonly, "last": lastpat}[kind]
            c = cut if kind == "ab" else cut_b
            res = []
            for w in range(2):
                items = pat[w][:c[w]] if first else pat[w][c[w]:]
                at = w * len(pattern[0]) + (0 if first else c[w]) if table and kind == "ab" else None
                res.append(kv_copies(t, items, last=kind == "last", tab_at=at))
            return res

        def issue(s, kind1, kind2, lo=0, hi=None):
            a, b = part(s + 1, kind1, False), part(s + 2, kind2, True)
            q0, q1 = a[0] + b[0], a[1] + b[1]
            for k, cp in enumerate(q0):
                cp._used = True
            for k, cp in enumerate(q1):
                cp._used = True
            start(q0[lo:hi], q1[lo:hi])

        def wait_a(u):
            wait_all(kva_v.at[u % nslots], sem_a.at[u % nslots])

        def wait_b(t):
            wait_all(kvb_v.at[t % nslots], sem_b.at[t % nslots])

        def out_copy(i, b):
            return pltpu.make_async_copy(out_v.at[b, :, pl.ds(i * D, D)], out_h.at[b, :, pl.ds(i * D, D)], sem_out)

        def big_out():
            if out_rows == 0:
                pltpu.make_async_copy(out_v.at[pl.ds(0, NB - 1)], out_h.at[pl.ds(0, NB - 1)],
                                      sem_out).start(priority=out_prio)
            else:
                k = 0
                for b in range(NB - 1):
                    for r in range(0, SQ, out_rows):
                        pltpu.make_async_copy(out_v.at[b, pl.ds(r, out_rows)], out_h.at[b, pl.ds(r, out_rows)],
                                              sem_out).start(priority=k % 2 if out_prio == 2 else out_prio)
                        k += 1

        def late_out(at):
            if out_mode == at:
                big_out()
                out_copy(0, NB - 1).start(priority=out_prio % 2)

        def softmax(s):
            m = jnp.max(s, axis=-1, keepdims=True)
            p = jnp.exp2(s - m)
            l = jnp.sum(p, axis=-1, keepdims=True)
            r = pltpu.reciprocal(l, approx=True)
            return p.astype(bf16), r * (2.0 - l * r)

        def heads(y):
            return [y[:, j * DH:(j + 1) * DH] for j in range(REP)]

        def group(u):
            return pl.ds(pl.multiple_of((u % G) * GW, GW), GW)

        def head(u, j):
            if hmap == 's':
                return pl.ds(pl.multiple_of((u % G + G * j) * DH, DH), DH)
            return pl.ds(pl.multiple_of(((u % G) * REP + j) * DH, DH), DH)

        def run(ops, ua, t, st=None, hooks=None):
            st = {} if st is None else st
            for op in ops.split():
                if hooks and op in hooks:
                    hooks[op]()
                if not compute:
                    continue
                i = 0 if op[1] == "a" else 1
                u = (ua, t)[i]
                slot = u % nslots
                if op[0] in "QN":
                    u = u + (op[0] == "N")
                    x = x_v[i, pl.ds(pl.multiple_of((u // G) * SQ, SQ), SQ), :]
                    if i and hmap == 's':
                        w = jnp.concatenate([wq_v[i, :, head(u, j)] for j in range(REP)], axis=1)
                    else:
                        w = wq_v[i, :, group(u)]
                    q = jnp.dot(x, w, preferred_element_type=f32)
                    st[op] = heads((q * QSCALE).astype(bf16))
                elif op == "Ka":
                    st[op] = lax.dot_general(jnp.concatenate(st["Qa"], axis=0), load(kva_v.at[slot, 0]), NT,
                                             preferred_element_type=f32)
                elif op[0] == "K":
                    j = int(op[1])
                    st[op] = lax.dot_general(st["Qb"][j], load(kvb_v.at[slot, 0, j]), NT,
                                             preferred_element_type=f32)
                elif op[0] == "S":
                    st[op] = softmax(st["K" + op[1]])
                elif op[0] == "V":
                    p, r = st["S" + op[1]]
                    v = load(kva_v.at[slot, 1] if i == 0 else kvb_v.at[slot, 1, int(op[1])])
                    st[op] = (jnp.dot(p, v, preferred_element_type=f32) * r).astype(bf16)
                elif op[0] == "O":
                    if i == 0:
                        o = [st["Va"][j * SQ:(j + 1) * SQ] for j in range(REP)]
                    else:
                        o = [st["V%d" % j] for j in range(REP)]
                    if i and hmap == 's':
                        w = jnp.concatenate([wo_v[i, head(u, j), :] for j in range(REP)], axis=0)
                    else:
                        w = wo_v[i, group(u), :]
                    y = jnp.dot(jnp.concatenate(o, axis=1), w, preferred_element_type=f32)
                    acc = jnp.where(u % G == 0, 0.0, acc_v[i]) + y
                    acc_v[i] = acc
                    out_v[u // G, :, i * D:(i + 1) * D] = acc.astype(bf16)
            return st

        nw = HW // 32
        per = nw // wstreams

        def w_loop(c):
            for k in range(wstreams):
                for i in range(2):
                    cc = k * per + (c + wstag * (4 * k + 2 * i)) % per
                    rows = pl.ds(pl.multiple_of((cc // 2) * 8, 8), 8)
                    cols = pl.ds(pl.multiple_of((cc % 2) * (HW // 2), HW // 2), HW // 2)
                    pltpu.make_async_copy(wq_h[i].at[rows, cols], wq_v.at[i, rows, cols], sem_w.at[1]).start(priority=0)
                    cc = k * per + (c + wstag * (4 * k + 2 * i + 1)) % per
                    rows = pl.ds(pl.multiple_of(cc * 32, 32), 32)
                    pltpu.make_async_copy(wo_h[i].at[rows], wo_v.at[i, rows], sem_w.at[2]).start(priority=1)

        with scope("wait_w"):
            pl.loop(0, per)(w_loop)
        for c in range(NB * SQ // 32):
            for i in range(2):
                pltpu.make_async_copy(x_h[i].at[pl.ds(c * 32, 32)], x_v.at[i, pl.ds(c * 32, 32)],
                                      sem_w.at[0]).start(priority=i)
        for u in range(ahead):
            start(*[kv_copies(u - ahead, [e for e in pattern[w] if e[0] < 2]) for w in range(2)])
        start(*part(0, "ab", True))
        issue(-1, "ab", "ab" if ahead == 1 else None)
        with scope("wait_z"):
            acc_v[...] = jnp.zeros_like(acc_v)
        wait_all(x_v, sem_w.at[0])
        wait_all(wq_v, sem_w.at[1])
        wait_all(wo_v, sem_w.at[2])

        def lead(u):
            with scope("wait"):
                wait_a(u)
            run(ORDER_A, u, None)

        if ahead == 1:
            lead(0)
        else:
            @pl.loop(0, ahead)
            def _(u):
                lead(u)

                @pl.when(u == 0)
                def _():
                    start(*part(1, "ab", True))

        @pl.loop(0, n - ahead)
        def _(s):
            with scope("wait"):
                wait_a(s + ahead)
                wait_b(s)

            with scope("issue"):
                m = n - ahead - 2

                @pl.when(s < m)
                def _():
                    issue(s, "ab", "ab", 0, mids[0][1] if mids else None)

                @pl.when(s == m)
                def _():
                    issue(m, "ab", "last" if ahead == 1 else "b")

                @pl.when(s == m + 1)
                def _():
                    issue(m + 1, *(("last", None) if ahead == 1 else ("b", "last")))

            hooks = {}
            for k, (op, lo) in enumerate(mids):
                def hook(lo=lo, hi=mids[k + 1][1] if k + 1 < len(mids) else None):
                    @pl.when(s < m)
                    def _():
                        issue(s, "ab", "ab", lo, hi)
                hooks[op] = hook
            run(order, s + ahead, s, hooks=hooks)

            if out_mode == "each":
                @pl.when((s + ahead) % G == G - 1)
                def _():
                    out_copy(0, (s + ahead) // G).start(priority=out_prio)

                @pl.when(s % G == G - 1)
                def _():
                    out_copy(1, s // G).start(priority=out_prio)
            elif isinstance(out_mode, int):
                @pl.when(s == out_mode)
                def _():
                    big_out()

        if isinstance(out_mode, int):
            out_copy(0, NB - 1).start(priority=out_prio % 2)
        late_out("loop")
        t = n - 1
        slot = t % nslots
        if ahead == 2:
            with scope("wait"):
                wait_b(n - 2)
            with scope("issue"):
                issue(n - 2, "last", None)
                late_out("issue")
            if early_q:
                st = run(ORDER_B.replace("V0", "Nb V0"), None, n - 2)
                st = {"Qb": st.get("Nb")}
            else:
                run(ORDER_B, None, n - 2)
                st = run("Qb", None, t)
        else:
            st = run("Qb", None, t)
        with scope("wait"):
            wait_all(kvb_v.at[slot, 0], sem_b.at[slot])
        late_out("k")
        run("K0 K1 K2 K3 S0 S1 S2 S3", None, t, st)
        acc = acc_v[1]
        for c, hs in enumerate(vgroups):
            with scope("wait"):
                wait_all(kvb_v.at[slot, 1, pl.ds(hs[0], len(hs))], sem_l.at[c])
            late_out("v%d" % c)
            run(" ".join("V%d" % h for h in hs), None, t, st)
            if compute:
                o = jnp.concatenate([st["V%d" % h] for h in hs], axis=1)
                w = jnp.concatenate([wo_v[1, head(t, h), :] for h in hs], axis=0)
                acc = acc + jnp.dot(o, w, preferred_element_type=f32)
        out_v[NB - 1, :, D:] = acc.astype(bf16)
        late_out("end")
        out_copy(1, NB - 1).start(priority=fin_prio)
        with scope("wait"):
            wait_all(out_v, sem_out)

    def fn(A_x, A_k, A_v, A_wq, A_wo, B_x, B_k, B_v, B_wq, B_wo, *tab):
        return pl.pallas_call(
            kernel,
            in_specs=[pl.BlockSpec(memory_space=pltpu.SMEM)] * len(tab) + [pl.BlockSpec(memory_space=pl.ANY)] * 10,
            out_specs=pl.BlockSpec(memory_space=pl.ANY),
            out_shape=jax.ShapeDtypeStruct((NB, SQ, 2 * D), bf16),
            scratch_shapes=[
                pltpu.VMEM((2, NB * SQ, D), bf16),
                pltpu.VMEM((2, D, HW), bf16),
                pltpu.VMEM((2, HW, D), bf16),
                pltpu.VMEM((nslots, 2, SK, DH), bf16),
                pltpu.VMEM((nslots, 2, REP, SK, DH), bf16),
                pltpu.VMEM((2, SQ, D), f32),
                pltpu.VMEM((NB, SQ, 2 * D), bf16),
                pltpu.SemaphoreType.DMA((4 + 2 * nslots + len(vgroups),)),
            ],
            compiler_params=pltpu.CompilerParams(vmem_limit_bytes=100 * MiB, disable_bounds_checks=True,
                                                 disable_semaphore_checks=True, flags=flags),
        )(*tab, A_x.reshape(NB * SQ, D), A_k, A_v, A_wq, A_wo, B_x.reshape(NB * SQ, D), B_k, B_v, B_wq, B_wo)
    return fn


_kernel_fn = make(wstreams=4, x0=24, out_mode='v0', hmap='s', pattern=default_pattern(0))


@jax.jit
def pallas_concat_heads__gqa_block_cached__mha_block_cached__near_ridge_kernel(
    A_x, A_k_cache, A_v_cache, A_wq, A_wo, B_x, B_k_cache, B_v_cache, B_wq, B_wo
):
    return _kernel_fn(A_x, A_k_cache, A_v_cache, A_wq, A_wo, B_x, B_k_cache, B_v_cache, B_wq, B_wo)
```

```python
import math

import jax
import jax.numpy as jnp
from jax import lax
import jax.experimental.pallas as pl
import jax.experimental.pallas.tpu as pltpu

BATCH, SQ, D_MODEL, SK, DH = 8, 48, 512, 1024, 128
GROUPS, REP = 8, 4
WIDTH = GROUPS * REP * DH
STEPS = BATCH * GROUPS
A, B = 0, 1
K, V = 0, 1

AHEAD = 2
SLOTS = 4

KV_ROWS = 128
KV_PIECES = SK // KV_ROWS
ROWS = 32
WEIGHT_PIECES = WIDTH // ROWS
WEIGHT_STREAMS = 2
QUEUE_LEAD = 24
LOOKAHEAD = 30
LAST_V = ((0, 1), (2,), (3,))

Q_SCALE = DH ** -0.5 * math.log2(math.e)


def _copy_plan():
    queues = ([], [])
    x_pieces = range(BATCH * SQ // ROWS)
    per_stream = WEIGHT_PIECES // WEIGHT_STREAMS
    queues[1].extend(("x", B, 0, p) for p in x_pieces)
    for p in range(per_stream):
        for stream in range(WEIGHT_STREAMS):
            for branch in (A, B):
                queues[0].append(("wq", branch, 0, stream * per_stream + p))
                queues[1].append(("wo", branch, 0, stream * per_stream + p))
    queues[0].extend(("x", A, 0, p) for p in x_pieces)
    for kv, streams in ((K, (0, 1, 2, 3, None)), (V, (0, 1, None, 2, 3))):
        for step in range(-AHEAD, STEPS - 1):
            for p in range(KV_PIECES):
                for head in streams:
                    if head is None and step + AHEAD < STEPS:
                        queues[kv].append(((A, kv), step, 0, p))
                    elif head is not None and step >= 0:
                        queues[kv].append(((B, kv), step, head, p))
    queues[K].extend(((B, K), STEPS - 1, h, p) for p in range(KV_PIECES) for h in range(REP))
    queues[V].extend(((B, V), STEPS - 1, h, p) for h in range(REP) for p in range(KV_PIECES))

    plan = [(1,) + copy for copy in queues[1][:QUEUE_LEAD]]
    for i, copy in enumerate(queues[0]):
        plan.append((0,) + copy)
        plan.extend((1,) + copy for copy in queues[1][i + QUEUE_LEAD:i + QUEUE_LEAD + 1])

    needed = {}
    for i, (_, array, step, _, _) in enumerate(plan):
        if not isinstance(array, str):
            needed[step] = i + 1
    windows, begin = {}, 0
    for step in range(-1, STEPS - 1):
        end = min(needed[step + 1] + LOOKAHEAD, len(plan))
        windows[step] = plan[begin:end]
        begin = end
        free = SLOTS - AHEAD if step < 0 else step + SLOTS
        assert all(isinstance(c[1], str) or c[2] < free for c in windows[step])
    assert begin == len(plan)
    return windows


def _kernel(xa_hbm, ka_hbm, va_hbm, wqa_hbm, woa_hbm, xb_hbm, kb_hbm, vb_hbm, wqb_hbm, wob_hbm,
            out_hbm, x_ref, wq_ref, wo_ref, kva_ref, kvb_ref, acc_ref, out_ref, last_ref, sems):
    sem_x, sem_wq, sem_wo, sem_out = (sems.at[i] for i in range(4))

    def sem_a(unit):
        return sems.at[4 + (unit & (SLOTS - 1))]

    def sem_b(unit):
        return sems.at[4 + SLOTS + (unit & (SLOTS - 1))]

    def sem_last_v(i):
        return sems.at[4 + 2 * SLOTS + i]

    def split(unit):
        return unit >> 3, unit & (GROUPS - 1), unit & (SLOTS - 1)

    def start(copies, base=0):
        for queue, array, index, head, piece in copies:
            if array == "x":
                rows = pl.ds(piece * ROWS, ROWS)
                src, dst, sem = (xa_hbm, xb_hbm)[index].at[rows], x_ref.at[index, rows], sem_x
            elif array == "wq":
                rows = pl.ds((piece // 2) * 8, 8)
                cols = pl.ds((piece % 2) * (WIDTH // 2), WIDTH // 2)
                src = (wqa_hbm, wqb_hbm)[index].at[rows, cols]
                dst, sem = wq_ref.at[index, rows, cols], sem_wq
            elif array == "wo":
                rows = pl.ds(piece * ROWS, ROWS)
                src, dst, sem = (woa_hbm, wob_hbm)[index].at[rows], wo_ref.at[index, rows], sem_wo
            else:
                branch, kv = array
                rows = pl.ds(piece * KV_ROWS, KV_ROWS)
                if branch == A:
                    unit = base + index + AHEAD
                    b, g, slot = split(unit)
                    src = (ka_hbm, va_hbm)[kv].at[b, g, rows]
                    dst, sem = kva_ref.at[slot, kv, rows], sem_a(unit)
                else:
                    unit = base + index
                    b, g, slot = split(unit)
                    src = (kb_hbm, vb_hbm)[kv].at[b, g + GROUPS * head, rows]
                    dst = kvb_ref.at[slot, kv, pl.ds(head * SK + piece * KV_ROWS, KV_ROWS)]
                    if kv == V and index == STEPS - 1:
                        sem = sem_last_v(next(i for i, hs in enumerate(LAST_V) if head in hs))
                    else:
                        sem = sem_b(unit)
            pltpu.make_async_copy(src, dst, sem).start(priority=queue)

    def wait_filled(ref, sem):
        pltpu.make_async_copy(ref, ref, sem).wait()

    def head_slice(branch, group, j):
        head = group * REP + j if branch == A else group + GROUPS * j
        return pl.ds(pl.multiple_of(head * DH, DH), DH)

    def project_q(branch, unit):
        b, g, _ = split(unit)
        x = x_ref[branch, pl.ds(pl.multiple_of(b * SQ, SQ), SQ), :]
        w = jnp.concatenate([wq_ref[branch, :, head_slice(branch, g, j)] for j in range(REP)], axis=1)
        q = (jnp.dot(x, w, preferred_element_type=jnp.float32) * Q_SCALE).astype(jnp.bfloat16)
        return [q[:, j * DH:(j + 1) * DH] for j in range(REP)]

    def scores(q, k):
        return lax.dot_general(q, k, (((1,), (1,)), ((), ())), preferred_element_type=jnp.float32)

    def softmax(s):
        p = jnp.exp2(s - jnp.max(s, axis=-1, keepdims=True))
        return p.astype(jnp.bfloat16), 1.0 / jnp.sum(p, axis=-1, keepdims=True)

    def weigh(probs, v):
        p, inv_sum = probs
        return (jnp.dot(p, v, preferred_element_type=jnp.float32) * inv_sum).astype(jnp.bfloat16)

    def project_out(branch, group, heads):
        o = jnp.concatenate(list(heads.values()), axis=1)
        w = jnp.concatenate([wo_ref[branch, head_slice(branch, group, j), :] for j in heads], axis=0)
        return jnp.dot(o, w, preferred_element_type=jnp.float32)

    def accumulate(branch, unit, outs):
        b, g, _ = split(unit)
        y = project_out(branch, g, dict(enumerate(outs)))
        acc = jnp.where(g == 0, 0.0, acc_ref[branch]) + y
        acc_ref[branch] = acc
        out_ref[b, :, branch * D_MODEL:(branch + 1) * D_MODEL] = acc.astype(jnp.bfloat16)

    def kv_a(unit, kv):
        return kva_ref[split(unit)[2], kv]

    def kv_b(unit, kv, j):
        return kvb_ref[split(unit)[2], kv, pl.ds(j * SK, SK)]

    def unstack(o):
        return [o[j * SQ:(j + 1) * SQ] for j in range(REP)]

    windows = _copy_plan()

    def relative(step):
        return [(q, a, i - step, h, p) for q, a, i, h, p in windows[step]]

    start(windows[-1])
    acc_ref[...] = jnp.zeros_like(acc_ref)
    wait_filled(x_ref, sem_x)
    wait_filled(wq_ref, sem_wq)
    wait_filled(wo_ref, sem_wo)

    @pl.loop(0, AHEAD)
    def _(unit):
        wait_filled(kva_ref.at[unit], sem_a(unit))
        s = scores(jnp.concatenate(project_q(A, unit), axis=0), kv_a(unit, K))
        accumulate(A, unit, unstack(weigh(softmax(s), kv_a(unit, V))))

    usual = relative(STEPS // 2)
    unusual = [step for step in range(STEPS - AHEAD) if relative(step) != usual]
    assert unusual == list(range(unusual[0], STEPS - AHEAD))

    @pl.loop(0, STEPS - AHEAD)
    def _(ub):
        ua = ub + AHEAD
        wait_filled(kva_ref.at[split(ua)[2]], sem_a(ua))
        wait_filled(kvb_ref.at[split(ub)[2]], sem_b(ub))
        pl.when(ub < unusual[0])(lambda: start(usual, ub))
        for step in unusual:
            pl.when(ub == step)(lambda: start(windows[step]))

        qb = project_q(B, ub)
        qa = project_q(A, ua)
        s0 = scores(qb[0], kv_b(ub, K, 0))
        s1 = scores(qb[1], kv_b(ub, K, 1))
        p0 = softmax(s0)
        sa = scores(jnp.concatenate(qa, axis=0), kv_a(ua, K))
        p1 = softmax(s1)
        o0 = weigh(p0, kv_b(ub, V, 0))
        s2 = scores(qb[2], kv_b(ub, K, 2))
        o1 = weigh(p1, kv_b(ub, V, 1))
        pa = softmax(sa)
        s3 = scores(qb[3], kv_b(ub, K, 3))
        p2 = softmax(s2)
        oa = weigh(pa, kv_a(ua, V))
        p3 = softmax(s3)
        o2 = weigh(p2, kv_b(ub, V, 2))
        o3 = weigh(p3, kv_b(ub, V, 3))
        accumulate(A, ua, unstack(oa))
        accumulate(B, ub, [o0, o1, o2, o3])

    last = STEPS - 1
    wait_filled(kvb_ref.at[split(last - 1)[2]], sem_b(last - 1))
    start(windows[last - 1])
    q = project_q(B, last - 1)
    s = [scores(q[j], kv_b(last - 1, K, j)) for j in range(REP)]
    p = [softmax(x) for x in s]
    q = project_q(B, last)
    accumulate(B, last - 1, [weigh(p[j], kv_b(last - 1, V, j)) for j in range(REP)])

    b, g, slot = split(last)
    wait_filled(kvb_ref.at[slot, K], sem_b(last))
    s = [scores(q[j], kv_b(last, K, j)) for j in range(REP)]
    p = [softmax(x) for x in s]
    writes = [
        pltpu.make_async_copy(out_ref.at[pl.ds(0, b)], out_hbm.at[pl.ds(0, b)], sem_out),
        pltpu.make_async_copy(out_ref.at[b, :, pl.ds(0, D_MODEL)],
                              out_hbm.at[b, :, pl.ds(0, D_MODEL)], sem_out),
        pltpu.make_async_copy(last_ref, out_hbm.at[b, :, pl.ds(D_MODEL, D_MODEL)], sem_out),
    ]
    acc = acc_ref[B]
    for i, heads in enumerate(LAST_V):
        wait_filled(kvb_ref.at[slot, V, pl.ds(heads[0] * SK, len(heads) * SK)], sem_last_v(i))
        if i == 0:
            writes[0].start(priority=1)
            writes[1].start(priority=1)
        acc = acc + project_out(B, g, {j: weigh(p[j], kv_b(last, V, j)) for j in heads})
    last_ref[...] = acc.astype(jnp.bfloat16)
    writes[2].start()
    for write in writes:
        write.wait()


@jax.jit
def pallas_concat_heads__gqa_block_cached__mha_block_cached__near_ridge_kernel(
    A_x: jax.Array,
    A_k_cache: jax.Array,
    A_v_cache: jax.Array,
    A_wq: jax.Array,
    A_wo: jax.Array,
    B_x: jax.Array,
    B_k_cache: jax.Array,
    B_v_cache: jax.Array,
    B_wq: jax.Array,
    B_wo: jax.Array,
):
    bf16 = jnp.bfloat16
    return pl.pallas_call(
        _kernel,
        in_specs=[pl.BlockSpec(memory_space=pl.ANY)] * 10,
        out_specs=pl.BlockSpec(memory_space=pl.ANY),
        out_shape=jax.ShapeDtypeStruct((BATCH, SQ, 2 * D_MODEL), bf16),
        scratch_shapes=[
            pltpu.VMEM((2, BATCH * SQ, D_MODEL), bf16),
            pltpu.VMEM((2, D_MODEL, WIDTH), bf16),
            pltpu.VMEM((2, WIDTH, D_MODEL), bf16),
            pltpu.VMEM((SLOTS, 2, SK, DH), bf16),
            pltpu.VMEM((SLOTS, 2, REP * SK, DH), bf16),
            pltpu.VMEM((2, SQ, D_MODEL), jnp.float32),
            pltpu.VMEM((BATCH, SQ, 2 * D_MODEL), bf16),
            pltpu.VMEM((SQ, D_MODEL), bf16),
            pltpu.SemaphoreType.DMA((4 + 2 * SLOTS + len(LAST_V),)),
        ],
        compiler_params=pltpu.CompilerParams(
            vmem_limit_bytes=64 << 20,
            disable_bounds_checks=True,
            disable_semaphore_checks=True,
        ),
    )(A_x.reshape(BATCH * SQ, D_MODEL), A_k_cache, A_v_cache, A_wq, A_wo,
      B_x.reshape(BATCH * SQ, D_MODEL), B_k_cache, B_v_cache, B_wq, B_wo)
```

```python
import math

import jax
import jax.numpy as jnp
from jax import lax
import jax.experimental.pallas as pl
import jax.experimental.pallas.tpu as pltpu

BATCH, SQ, D_MODEL, SK, DH = 8, 48, 512, 1024, 128
GROUPS, REP = 8, 4
WIDTH = GROUPS * REP * DH
STEPS = BATCH * GROUPS
A, B = 0, 1
K, V = 0, 1

AHEAD = 2
SLOTS = 4

KV_ROWS = 128
KV_PIECES = SK // KV_ROWS
ROWS = 32
WEIGHT_PIECES = WIDTH // ROWS
WEIGHT_STREAMS = 2
QUEUE_LEAD = 24
LOOKAHEAD = 30
LAST_READS = 10

Q_SCALE = DH ** -0.5 * math.log2(math.e)


def _copy_plan():
    queues = ([], [])
    x_pieces = range(BATCH * SQ // ROWS)
    per_stream = WEIGHT_PIECES // WEIGHT_STREAMS
    queues[1].extend(("x", B, 0, p) for p in x_pieces)
    for p in range(per_stream):
        for stream in range(WEIGHT_STREAMS):
            for branch in (A, B):
                queues[0].append(("wq", branch, 0, stream * per_stream + p))
                queues[1].append(("wo", branch, 0, stream * per_stream + p))
    queues[0].extend(("x", A, 0, p) for p in x_pieces)
    for kv, streams in ((K, (0, 1, 2, 3, None)), (V, (0, 1, None, 2, 3))):
        for step in range(-AHEAD, STEPS - 1):
            for p in range(KV_PIECES):
                for head in streams:
                    if head is None and step + AHEAD < STEPS:
                        queues[kv].append(((A, kv), step, 0, p))
                    elif head is not None and step >= 0:
                        queues[kv].append(((B, kv), step, head, p))
    queues[K].extend(((B, K), STEPS - 1, h, p) for p in range(KV_PIECES) for h in range(REP))
    queues[V].extend(((B, V), STEPS - 1, h, p) for h in range(REP) for p in range(KV_PIECES))

    plan = [(1,) + copy for copy in queues[1][:QUEUE_LEAD]]
    for i, copy in enumerate(queues[0]):
        plan.append((0,) + copy)
        plan.extend((1,) + copy for copy in queues[1][i + QUEUE_LEAD:i + QUEUE_LEAD + 1])

    needed = {}
    for i, (_, array, step, _, _) in enumerate(plan):
        if not isinstance(array, str):
            needed[step] = i + 1
    windows, begin = {}, 0
    for step in range(-1, STEPS - 1):
        end = min(needed[step + 1] + LOOKAHEAD, len(plan))
        windows[step] = plan[begin:end]
        begin = end
        free = SLOTS - AHEAD if step < 0 else step + SLOTS
        assert all(isinstance(c[1], str) or c[2] < free for c in windows[step])
    assert begin == len(plan)
    return windows


def _kernel(xa_hbm, ka_hbm, va_hbm, wqa_hbm, woa_hbm, xb_hbm, kb_hbm, vb_hbm, wqb_hbm, wob_hbm,
            out_hbm, x_ref, wq_ref, wo_ref, kva_ref, kvb_ref, acc_ref, out_ref, last_ref, sems):
    sem_x, sem_wq, sem_wo, sem_out, sem_v_early, sem_v_late = (sems.at[i] for i in range(6))
    early_rows = (REP * KV_PIECES - LAST_READS) * KV_ROWS

    def sem_a(unit):
        return sems.at[6 + (unit & (SLOTS - 1))]

    def sem_b(unit):
        return sems.at[6 + SLOTS + (unit & (SLOTS - 1))]

    def split(unit):
        return unit >> 3, unit & (GROUPS - 1), unit & (SLOTS - 1)

    def start(copies, base=0):
        for queue, array, index, head, piece in copies:
            if array == "x":
                rows = pl.ds(piece * ROWS, ROWS)
                src, dst, sem = (xa_hbm, xb_hbm)[index].at[rows], x_ref.at[index, rows], sem_x
            elif array == "wq":
                rows = pl.ds((piece // 2) * 8, 8)
                cols = pl.ds((piece % 2) * (WIDTH // 2), WIDTH // 2)
                src = (wqa_hbm, wqb_hbm)[index].at[rows, cols]
                dst, sem = wq_ref.at[index, rows, cols], sem_wq
            elif array == "wo":
                rows = pl.ds(piece * ROWS, ROWS)
                src, dst, sem = (woa_hbm, wob_hbm)[index].at[rows], wo_ref.at[index, rows], sem_wo
            else:
                branch, kv = array
                rows = pl.ds(piece * KV_ROWS, KV_ROWS)
                if branch == A:
                    unit = base + index + AHEAD
                    b, g, slot = split(unit)
                    src = (ka_hbm, va_hbm)[kv].at[b, g, rows]
                    dst, sem = kva_ref.at[slot, kv, rows], sem_a(unit)
                else:
                    unit = base + index
                    b, g, slot = split(unit)
                    src = (kb_hbm, vb_hbm)[kv].at[b, g + GROUPS * head, rows]
                    row = head * SK + piece * KV_ROWS
                    dst = kvb_ref.at[slot, kv, pl.ds(row, KV_ROWS)]
                    if kv == V and index == STEPS - 1:
                        sem = sem_v_early if row < early_rows else sem_v_late
                    else:
                        sem = sem_b(unit)
            pltpu.make_async_copy(src, dst, sem).start(priority=queue)

    def wait_filled(ref, sem):
        pltpu.make_async_copy(ref, ref, sem).wait()

    def head_slice(branch, group, j):
        head = group * REP + j if branch == A else group + GROUPS * j
        return pl.ds(pl.multiple_of(head * DH, DH), DH)

    def project_q(branch, unit):
        b, g, _ = split(unit)
        x = x_ref[branch, pl.ds(pl.multiple_of(b * SQ, SQ), SQ), :]
        w = jnp.concatenate([wq_ref[branch, :, head_slice(branch, g, j)] for j in range(REP)], axis=1)
        q = (jnp.dot(x, w, preferred_element_type=jnp.float32) * Q_SCALE).astype(jnp.bfloat16)
        return [q[:, j * DH:(j + 1) * DH] for j in range(REP)]

    def scores(q, k):
        return lax.dot_general(q, k, (((1,), (1,)), ((), ())), preferred_element_type=jnp.float32)

    def softmax(s):
        p = jnp.exp2(s - jnp.max(s, axis=-1, keepdims=True))
        return p.astype(jnp.bfloat16), 1.0 / jnp.sum(p, axis=-1, keepdims=True)

    def weigh(probs, v):
        p, inv_sum = probs
        return (jnp.dot(p, v, preferred_element_type=jnp.float32) * inv_sum).astype(jnp.bfloat16)

    def project_out(branch, group, heads):
        o = jnp.concatenate(list(heads.values()), axis=1)
        w = jnp.concatenate([wo_ref[branch, head_slice(branch, group, j), :] for j in heads], axis=0)
        return jnp.dot(o, w, preferred_element_type=jnp.float32)

    def accumulate(branch, unit, outs):
        b, g, _ = split(unit)
        y = project_out(branch, g, dict(enumerate(outs)))
        acc = jnp.where(g == 0, 0.0, acc_ref[branch]) + y
        acc_ref[branch] = acc
        out_ref[b, :, branch * D_MODEL:(branch + 1) * D_MODEL] = acc.astype(jnp.bfloat16)

    def kv_a(unit, kv):
        return kva_ref[split(unit)[2], kv]

    def kv_b(unit, kv, j):
        return kvb_ref[split(unit)[2], kv, pl.ds(j * SK, SK)]

    def unstack(o):
        return [o[j * SQ:(j + 1) * SQ] for j in range(REP)]

    windows = _copy_plan()

    def relative(step):
        return [(q, a, i - step, h, p) for q, a, i, h, p in windows[step]]

    start(windows[-1])
    acc_ref[...] = jnp.zeros_like(acc_ref)
    wait_filled(x_ref, sem_x)
    wait_filled(wq_ref, sem_wq)
    wait_filled(wo_ref, sem_wo)

    @pl.loop(0, AHEAD)
    def _(unit):
        wait_filled(kva_ref.at[unit], sem_a(unit))
        s = scores(jnp.concatenate(project_q(A, unit), axis=0), kv_a(unit, K))
        accumulate(A, unit, unstack(weigh(softmax(s), kv_a(unit, V))))

    usual = relative(STEPS // 2)
    unusual = [step for step in range(STEPS - AHEAD) if relative(step) != usual]
    assert unusual == list(range(unusual[0], STEPS - AHEAD))

    @pl.loop(0, STEPS - AHEAD)
    def _(ub):
        ua = ub + AHEAD
        wait_filled(kva_ref.at[split(ua)[2]], sem_a(ua))
        wait_filled(kvb_ref.at[split(ub)[2]], sem_b(ub))
        pl.when(ub < unusual[0])(lambda: start(usual, ub))
        for step in unusual:
            pl.when(ub == step)(lambda: start(windows[step]))

        qb = project_q(B, ub)
        qa = project_q(A, ua)
        s0 = scores(qb[0], kv_b(ub, K, 0))
        s1 = scores(qb[1], kv_b(ub, K, 1))
        p0 = softmax(s0)
        sa = scores(jnp.concatenate(qa, axis=0), kv_a(ua, K))
        p1 = softmax(s1)
        o0 = weigh(p0, kv_b(ub, V, 0))
        s2 = scores(qb[2], kv_b(ub, K, 2))
        o1 = weigh(p1, kv_b(ub, V, 1))
        pa = softmax(sa)
        s3 = scores(qb[3], kv_b(ub, K, 3))
        p2 = softmax(s2)
        oa = weigh(pa, kv_a(ua, V))
        p3 = softmax(s3)
        o2 = weigh(p2, kv_b(ub, V, 2))
        o3 = weigh(p3, kv_b(ub, V, 3))
        accumulate(A, ua, unstack(oa))
        accumulate(B, ub, [o0, o1, o2, o3])

    last = STEPS - 1
    wait_filled(kvb_ref.at[split(last - 1)[2]], sem_b(last - 1))
    start(windows[last - 1])
    q = project_q(B, last - 1)
    s = [scores(q[j], kv_b(last - 1, K, j)) for j in range(REP)]
    p = [softmax(x) for x in s]
    q = project_q(B, last)
    accumulate(B, last - 1, [weigh(p[j], kv_b(last - 1, V, j)) for j in range(REP)])

    b, g, slot = split(last)
    wait_filled(kvb_ref.at[slot, K], sem_b(last))
    s = [scores(q[j], kv_b(last, K, j)) for j in range(REP)]
    p = [softmax(x) for x in s]
    writes = [
        pltpu.make_async_copy(out_ref.at[pl.ds(0, b)], out_hbm.at[pl.ds(0, b)], sem_out),
        pltpu.make_async_copy(out_ref.at[b, :, pl.ds(0, D_MODEL)],
                              out_hbm.at[b, :, pl.ds(0, D_MODEL)], sem_out),
        pltpu.make_async_copy(last_ref, out_hbm.at[b, :, pl.ds(D_MODEL, D_MODEL)], sem_out),
    ]

    def finish(heads):
        return project_out(B, g, {j: weigh(p[j], kv_b(last, V, j)) for j in heads})

    early_heads = early_rows // SK
    wait_filled(kvb_ref.at[slot, V, pl.ds(0, early_rows)], sem_v_early)
    writes[0].start(priority=1)
    writes[1].start(priority=1)
    acc = acc_ref[B] + finish(range(early_heads))
    wait_filled(kvb_ref.at[slot, V, pl.ds(early_rows, REP * SK - early_rows)], sem_v_late)
    acc = acc + finish(range(early_heads, REP))
    last_ref[...] = acc.astype(jnp.bfloat16)
    writes[2].start()
    for write in writes:
        write.wait()


@jax.jit
def pallas_concat_heads__gqa_block_cached__mha_block_cached__near_ridge_kernel(
    A_x: jax.Array,
    A_k_cache: jax.Array,
    A_v_cache: jax.Array,
    A_wq: jax.Array,
    A_wo: jax.Array,
    B_x: jax.Array,
    B_k_cache: jax.Array,
    B_v_cache: jax.Array,
    B_wq: jax.Array,
    B_wo: jax.Array,
):
    bf16 = jnp.bfloat16
    return pl.pallas_call(
        _kernel,
        in_specs=[pl.BlockSpec(memory_space=pl.ANY)] * 10,
        out_specs=pl.BlockSpec(memory_space=pl.ANY),
        out_shape=jax.ShapeDtypeStruct((BATCH, SQ, 2 * D_MODEL), bf16),
        scratch_shapes=[
            pltpu.VMEM((2, BATCH * SQ, D_MODEL), bf16),
            pltpu.VMEM((2, D_MODEL, WIDTH), bf16),
            pltpu.VMEM((2, WIDTH, D_MODEL), bf16),
            pltpu.VMEM((SLOTS, 2, SK, DH), bf16),
            pltpu.VMEM((SLOTS, 2, REP * SK, DH), bf16),
            pltpu.VMEM((2, SQ, D_MODEL), jnp.float32),
            pltpu.VMEM((BATCH, SQ, 2 * D_MODEL), bf16),
            pltpu.VMEM((SQ, D_MODEL), bf16),
            pltpu.SemaphoreType.DMA((6 + 2 * SLOTS,)),
        ],
        compiler_params=pltpu.CompilerParams(
            vmem_limit_bytes=64 << 20,
            disable_bounds_checks=True,
            disable_semaphore_checks=True,
        ),
    )(A_x.reshape(BATCH * SQ, D_MODEL), A_k_cache, A_v_cache, A_wq, A_wo,
      B_x.reshape(BATCH * SQ, D_MODEL), B_k_cache, B_v_cache, B_wq, B_wo)
```
